```python
import os as _os
_os.environ.setdefault("JAX_PLATFORMS", "cpu")
import jax
import jax.numpy as jnp

def _softmax(x, axis=-1):
    return jax.nn.softmax(x, axis=axis)
def _gelu(x):
    return jax.nn.gelu(x, approximate=True)
def _silu(x):
    return jax.nn.silu(x)
def _sigmoid(x):
    return jax.nn.sigmoid(x)
def _layernorm(x, axis=-1, eps=1e-5):
    m = jnp.mean(x, axis=axis, keepdims=True)
    v = jnp.var(x, axis=axis, keepdims=True)
    return (x - m) / jnp.sqrt(v + eps)
def _scatter_add(tgt, idx, src, axis=0):
    return tgt.at[idx].add(src)
def _segment_sum(src, seg, n):
    return jax.ops.segment_sum(src, seg, n)
class _Rng:
    def __init__(self, key):
        self._k = key
    def _next(self):
        self._k, sub = jax.random.split(self._k)
        return sub
    def normal(self, shape):
        return jax.random.normal(self._next(), shape, dtype=jnp.bfloat16)
    def randint(self, lo, hi, shape):
        return jax.random.randint(self._next(), shape, lo, hi, dtype=jnp.int32)
    def uniform(self, shape, lo=0.0, hi=1.0):
        return jax.random.uniform(self._next(), shape, jnp.bfloat16, lo, hi)
    def permutation(self, n):
        return jax.random.permutation(self._next(), n)


kernel_name = 'parallel_sum__sliding_local_dilated__glu_gated_geglu__prompt'

def setup_inputs():
    _rng = _Rng(jax.random.key(int.from_bytes(__import__("os").urandom(4), "little")))
    _w = (lambda a: (lambda t: t.astype(jnp.bfloat16) if jnp.issubdtype(t.dtype, jnp.floating) else t)(jnp.asarray(a)))
    def _A_setup():
        B, S, D = 1, 2048, 512
        return {
            "x": _w((lambda *s: _rng.normal(s) * 0.05)(B, S, D)),
            "wqkv": _w((lambda *s: _rng.normal(s) * 0.05)(D, 3 * D)),
            "wo": _w((lambda *s: _rng.normal(s) * 0.05)(D, D)),
        }
    _A_in = _A_setup()

    def _B_setup():
        B, S, Dm, Df = 1, 2048, 512, 1376
        return {
            "x": _w((lambda *s: _rng.normal(s) * 0.05)(B, S, Dm)),
            "w_gate": _w((lambda *s: _rng.normal(s) * 0.1)(Dm, Df) * (Dm ** -0.5)),
            "w_up": _w((lambda *s: _rng.normal(s) * 0.1)(Dm, Df) * (Dm ** -0.5)),
            "w_down": _w((lambda *s: _rng.normal(s) * 0.1)(Df, Dm) * (Df ** -0.5)),
        }
    _B_in = _B_setup()

    return {
        "A_x": _A_in["x"],
        "A_wqkv": _A_in["wqkv"],
        "A_wo": _A_in["wo"],
        "B_x": _B_in["x"],
        "B_w_gate": _B_in["w_gate"],
        "B_w_up": _B_in["w_up"],
        "B_w_down": _B_in["w_down"],
    }

def reference(A_x, A_wqkv, A_wo, B_x, B_w_gate, B_w_up, B_w_down):
    def _A_ref(x, wqkv, wo):
        B, S, D = x.shape
        H = 32; Dh = D // H
        W, dil = 8, 2
        qkv = (lambda x, *d: x.transpose(*d))((x @ wqkv).reshape(B, S, 3, H, Dh), 2, 0, 3, 1, 4)
        q, k, v = qkv[0], qkv[1], qkv[2]
        scale = Dh ** -0.5
        pos = jnp.arange(S)
        off = jnp.arange(W) * dil
        idx = pos[:, None] - off[None, :]
        mask = idx >= 0
        idx_c = jnp.where(mask, idx, 0).reshape(-1)
        kg = k[:, :, idx_c, :].reshape(B, H, S, W, Dh)
        vg = v[:, :, idx_c, :].reshape(B, H, S, W, Dh)
        logits = jnp.einsum("bhsd,bhswd->bhsw", q, kg) * scale
        logits = jnp.where(mask[None, None, :, :], logits, -1e9)
        attn = _softmax(logits, axis=-1)
        o = jnp.einsum("bhsw,bhswd->bhsd", attn, vg)
        return (lambda x, *d: x.transpose(*d))(o, 0, 2, 1, 3).reshape(B, S, D) @ wo

    def _B_ref(x, w_gate, w_up, w_down):
        g = jnp.einsum("bsd,df->bsf", x, w_gate)
        u = jnp.einsum("bsd,df->bsf", x, w_up)
        h = _gelu(g) * u
        return jnp.einsum("bsf,fd->bsd", h, w_down)

    x = A_x
    xn = _layernorm(x, axis=-1)
    return x + _A_ref(xn, A_wqkv, A_wo) + _B_ref(xn, B_w_gate, B_w_up, B_w_down)
```

```python
import functools
import numpy as np
import jax
import jax.numpy as jnp
from jax import lax
import jax.experimental.pallas as pl
import jax.experimental.pallas.tpu as pltpu

S, D, H, DH, W, DIL, DF = 2048, 512, 32, 16, 8, 2, 1376
NF = 11
DFP = NF * 128
HALO = 16
LOG2E = 1.4426950408889634
F32 = jnp.float32
BF = jnp.bfloat16
U32 = jnp.uint32
NT_DIMS = (((1,), (1,)), ((), ()))
SCOPES = False
T0MAX = 512


def cat(xs):
    return jnp.concatenate(xs, axis=1)


def _kernel(x_hbm, wqkv_hbm, wo_hbm, wg_hbm, wu_hbm, wd_hbm, o_hbm,
            x_buf, o_buf, xn_buf, xn2_buf, h_buf, wqkv_raw, wt_p, wo_raw, stage0, stage1, stage2, stage3, wo_p,
            wg_v, wu_v, wd_v, q_scr, k_scr, v_scr, sems, osem, *, prog, FIN):
    sem_i = [0]
    cps = {}

    def group(name, pairs):
        sem = sems.at[sem_i[0]]
        sem_i[0] += 1
        cps[name] = [pltpu.make_async_copy(a, b, sem) for a, b in pairs]
        for c in cps[name]:
            c.start()

    def x_pairs(a, n):
        return [(x_hbm.at[pl.ds(a, n)], x_buf.at[pl.ds(a, n)])]

    def w_pairs(src, dst, a, n):
        return [(src.at[pl.ds(a, n)], dst.at[pl.ds(a, n)])]

    def start(name, *items):
        pairs = []
        for it in items:
            if it[0] == "x":
                pairs += x_pairs(it[1], it[2])
            elif it[0] == "g":
                pairs += w_pairs(wg_hbm, wg_v, it[1], it[2])
            elif it[0] == "u":
                pairs += w_pairs(wu_hbm, wu_v, it[1], it[2])
            elif it[0] == "d":
                pairs += w_pairs(wd_hbm, wd_v, it[1], it[2])
            elif it[0] == "qkv":
                pairs.append((wqkv_hbm, wqkv_raw))
            elif it[0] == "wo":
                pairs.append((wo_hbm, wo_raw))
        group(name, pairs)

    def wait(name):
        for c in cps.pop(name):
            c.wait()

    def ocopy(r, n):
        return pltpu.make_async_copy(o_buf.at[pl.ds(r, n)], o_hbm.at[pl.ds(r, n)], osem.at[0])

    def st_o(r, n):
        ocopy(r, n).start()

    def wait_o(r, n):
        ocopy(r, n).wait()

    def _ln(r0, n):
        x = x_buf[pl.ds(r0, n), :].astype(F32)
        mu = jnp.sum(x, axis=-1, keepdims=True) * (1.0 / D)
        xc = x - mu
        var = jnp.sum(xc * xc, axis=-1, keepdims=True) * (1.0 / D)
        return (xc * lax.rsqrt(var + 1e-5)).astype(BF)

    def ln(r0, n, l0):
        xn_buf[pl.ds(l0, n), :] = _ln(r0, n)

    def ln2(r0, n):
        xn2_buf[pl.ds(0, n), :] = _ln(r0, n)

    def xcopy(n):
        xn_buf[pl.ds(0, n), :] = xn2_buf[pl.ds(0, n), :]

    def get_xn(l0, n):
        return xn_buf[pl.ds(l0, n), :]

    def _act(g, u):
        inner = g * (0.7978845608028654 + (0.7978845608028654 * 0.044715) * (g * g))
        hg = 0.5 * g
        return ((hg + hg * jnp.tanh(inner)) * u).astype(BF)

    def gu(l0, n, a, m):
        xn = get_xn(l0, n)
        g = lax.dot_general(xn, wg_v[pl.ds(a, m), :], NT_DIMS, preferred_element_type=F32)
        u = lax.dot_general(xn, wu_v[pl.ds(a, m), :], NT_DIMS, preferred_element_type=F32)
        h_buf[pl.ds(l0, n), pl.ds(a, m)] = _act(g, u)

    def _row_perm(wv, dst, base, stage):
        for j in range(4):
            stage[j] = wv[:, 128 * j:128 * (j + 1)]
        for e in range(8):
            A = cat([stage[j, pl.ds(e, 16, stride=16), :] for j in range(4)])
            B = cat([stage[j, pl.ds(8 + e, 16, stride=16), :] for j in range(4)])
            lo = (A & 0xFFFF) | (B << 16)
            hi = lax.shift_right_logical(A, U32(16)) | (B & U32(0xFFFF0000))
            dst[pl.ds(base + 64 * e, 32), :] = pltpu.bitcast(lo, BF)
            dst[pl.ds(base + 64 * e + 32, 32), :] = pltpu.bitcast(hi, BF)

    def prep_qkv(s):
        wt = wqkv_raw[:, pl.ds(D * s, D)].T
        _row_perm(pltpu.bitcast(wt, U32), wt_p, D * s, (stage0, stage1, stage2)[s])

    def prep_wo():
        _row_perm(pltpu.bitcast(wo_raw[...], U32), wo_p, 0, stage3)

    def qkv(l0, n, first):
        xn = get_xn(l0, n)
        r = lax.dot_general(xn, wt_p[...], NT_DIMS, preferred_element_type=F32)
        sc = (DH ** -0.5) * LOG2E
        for j in range(4):
            q_scr[j, pl.ds(l0, n), :] = r[:, 128 * j:128 * (j + 1)] * sc
            k_scr[j, pl.ds(HALO + l0, n), :] = r[:, D + 128 * j:D + 128 * (j + 1)]
            v_scr[j, pl.ds(HALO + l0, n), :] = r[:, 2 * D + 128 * j:2 * D + 128 * (j + 1)]
        if first:
            for j in range(4):
                k_scr[j, 0:HALO, :] = jnp.zeros((HALO, 128), F32)
                v_scr[j, 0:HALO, :] = jnp.broadcast_to(r[0:1, 2 * D + 128 * j:2 * D + 128 * (j + 1)], (HALO, 128))

    def halo(lsrc):
        for j in range(4):
            k_scr[j, 0:HALO, :] = k_scr[j, pl.ds(lsrc, HALO), :]
            v_scr[j, 0:HALO, :] = v_scr[j, pl.ds(lsrc, HALO), :]

    oa_val = {}

    def attn(l0, n, first):
        q = [q_scr[j, pl.ds(l0, n), :] for j in range(4)]
        lg = []
        base = HALO + l0
        for w in range(W):
            s = None
            for j in range(4):
                p = q[j] * k_scr[j, pl.ds(base - DIL * w, n), :]
                s = p if s is None else s + p
            s = s + pltpu.roll(s, 64, 1)
            s = s + pltpu.roll(s, 32, 1)
            if w > 0 and first:
                pos = lax.broadcasted_iota(jnp.int32, (HALO, 128), 0)
                top = jnp.where(pos >= DIL * w, s[0:HALO], -1e9 * LOG2E)
                s = jnp.concatenate([top, s[HALO:]], axis=0)
            lg.append(s)
        m = lg[0]
        for w in range(1, W):
            m = jnp.maximum(m, lg[w])
        e = [jnp.exp2(l - m) for l in lg]
        den = e[0]
        for w in range(1, W):
            den = den + e[w]
        inv = 1.0 / den
        oo = []
        for j in range(4):
            a = None
            for w in range(W):
                tt = e[w] * v_scr[j, pl.ds(base - DIL * w, n), :]
                a = tt if a is None else a + tt
            oo.append((a * inv).astype(BF))
        oa_val[l0] = cat(oo)

    def fin(r0, n, l0):
        if FIN == 0:
            acc = jnp.dot(h_buf[pl.ds(l0, n), :], wd_v[...], preferred_element_type=F32)
            acc = acc + jnp.dot(oa_val.pop(l0), wo_p[...], preferred_element_type=F32)
            x = x_buf[pl.ds(r0, n), :].astype(F32)
            o_buf[pl.ds(r0, n), :] = (x + acc).astype(BF)
        elif FIN == 1:
            acc = jnp.dot(oa_val.pop(l0), wo_p[...], preferred_element_type=F32)
            acc = acc + jnp.dot(h_buf[pl.ds(l0, n), :], wd_v[...], preferred_element_type=F32)
            x = x_buf[pl.ds(r0, n), :].astype(F32)
            o_buf[pl.ds(r0, n), :] = (x + acc).astype(BF)
        else:
            x = x_buf[pl.ds(r0, n), :].astype(F32)
            acc = x + jnp.dot(h_buf[pl.ds(l0, n), :], wd_v[...], preferred_element_type=F32)
            acc = acc + jnp.dot(oa_val.pop(l0), wo_p[...], preferred_element_type=F32)
            o_buf[pl.ds(r0, n), :] = acc.astype(BF)

    scope = [None]

    def mark(name):
        if scope[0] is not None:
            scope[0].__exit__(None, None, None)
            scope[0] = None
        if name:
            scope[0] = jax.named_scope(name)
            scope[0].__enter__()

    def loop(r_start, niter, step, body):
        def it(i, c):
            r = pl.multiple_of(r_start + i * step, step)
            ops = [(op[0], [subst(z, r, i) for z in op[1:]]) for op in body]
            if SCOPES:
                with jax.named_scope("ITER"):
                    for name, args in ops:
                        env[name](*args)
            else:
                for name, args in ops:
                    env[name](*args)
            return c
        lax.fori_loop(0, niter, it, 0)

    def subst(z, r, i):
        if isinstance(z, tuple) and z and z[0] == "R":
            return pl.multiple_of(r + z[1], 16)
        if isinstance(z, tuple) and z and z[0] == "RC":
            return pl.multiple_of(jnp.minimum(r + z[1], z[2]), 16)
        return z

    env = dict(start=start, wait=wait, st_o=st_o, wait_o=wait_o, ln=ln, ln2=ln2, xcopy=xcopy, gu=gu,
               prep_qkv=prep_qkv, prep_wo=prep_wo, qkv=qkv, attn=attn, fin=fin, halo=halo, loop=loop,
               mark=mark)
    if SCOPES:
        newp = []
        for k, op in enumerate(prog):
            newp.append(op)
            if op[0] in ("wait", "st_o", "wait_o", "loop") and (k + 1 == len(prog) or prog[k + 1][0] not in ("wait", "wait_o")):
                newp.append(("mark", "R%02d_%s" % (k, op[1])))
        newp.append(("mark", None))
        prog = newp
    for op in prog:
        env[op[0]](*op[1:])
    assert not cps, list(cps)


def prog_loop(T=256, chunks=(256, 384, 384, 352), T0=512, unroll=1):
    P = []
    ch = []
    a = 0
    for m in chunks:
        ch.append((a, m)); a += m
    assert a == DF
    NC = len(ch)
    P.append(("start", "x0", ("x", 0, T0)))
    for i, (a, m) in enumerate(ch):
        P.append(("start", "c%d" % i, ("g", a, m), ("u", a, m)))
    P.append(("start", "qkv", ("qkv",)))
    P.append(("start", "rest", ("wo",), ("d", 0, DF), ("x", T0, S - T0)))
    P += [("wait", "x0"), ("ln", 0, T0, 0)]
    for i, (a, m) in enumerate(ch):
        P.append(("wait", "c%d" % i))
        if i == NC - 1:
            P.append(("wait", "qkv"))
        P.append(("gu", 0, T0, a, m))
    P += [("prep_qkv", 0), ("prep_qkv", 1), ("prep_qkv", 2)]
    tiles0 = list(range(0, T0, T))
    P.append(("qkv", 0, T, True))
    P += [("wait", "rest"), ("prep_wo",)]
    for r in tiles0[1:]:
        P.append(("qkv", r, T, False))
    for r in tiles0:
        P.append(("attn", r, T, r == 0))
    P.append(("halo", T0))
    P.append(("ln", T0, T, 0))
    for r in tiles0:
        P.append(("fin", r, T, r))
    P.append(("st_o", 0, T0))
    n = (S - T0) // T
    body = []
    for u in range(unroll):
        body += [("ln2", ("RC", u * T + T, S - T), T), ("qkv", 0, T, False), ("attn", 0, T, False), ("gu", 0, T, 0, DF),
                 ("halo", T), ("xcopy", T), ("fin", ("R", u * T), T, 0), ("st_o", ("R", u * T), T)]
    P.append(("loop", T0, n // unroll, T * unroll, body))
    P.append(("wait_o", 0, T0))
    for i in range(n):
        P.append(("wait_o", T0 + i * T, T))
    return P


def _make(prog="prog_loop", flags=None, nosemchk=False, FIN=0, **kw):
    prog = prog_loop(**kw)
    nsem = sum(1 for op in prog if op[0] == "start")

    @jax.jit
    def fn(A_x, A_wqkv, A_wo, B_x, B_w_gate, B_w_up, B_w_down):
        x = A_x.reshape(S, D)
        hbm = pl.BlockSpec(memory_space=pltpu.HBM)
        out = pl.pallas_call(
            functools.partial(_kernel, prog=prog, FIN=FIN),
            in_specs=[hbm] * 6,
            out_specs=hbm,
            out_shape=jax.ShapeDtypeStruct((S, D), A_x.dtype),
            scratch_shapes=[
                pltpu.VMEM((S, D), BF), pltpu.VMEM((S, D), BF),
                pltpu.VMEM((T0MAX, D), BF), pltpu.VMEM((T0MAX, D), BF),
                pltpu.VMEM((T0MAX, DF), BF),
                pltpu.VMEM((D, 3 * D), BF), pltpu.VMEM((3 * D, D), BF),
                pltpu.VMEM((D, D), BF)] + [pltpu.VMEM((4, D // 2, 128), U32)] * 4 + [
                pltpu.VMEM((D, D), BF),
                pltpu.VMEM((DF, D), BF), pltpu.VMEM((DF, D), BF), pltpu.VMEM((DF, D), BF),
                pltpu.VMEM((4, T0MAX, 128), F32),
                pltpu.VMEM((4, HALO + T0MAX, 128), F32), pltpu.VMEM((4, HALO + T0MAX, 128), F32),
                pltpu.SemaphoreType.DMA((nsem,)), pltpu.SemaphoreType.DMA((1,)),
            ],
            compiler_params=pltpu.CompilerParams(vmem_limit_bytes=110 * 1024 * 1024, flags=flags,
                                                 disable_semaphore_checks=nosemchk),
        )(x, A_wqkv, A_wo, B_w_gate.T, B_w_up.T, B_w_down)
        return out.reshape(1, S, D)
    return fn


_fn = _make(FIN=1,unroll=2)


@jax.jit
def pallas_parallel_sum__sliding_local_dilated__glu_gated_geglu__prompt_kernel(
    A_x: jax.Array,
    A_wqkv: jax.Array,
    A_wo: jax.Array,
    B_x: jax.Array,
    B_w_gate: jax.Array,
    B_w_up: jax.Array,
    B_w_down: jax.Array,
):
    return _fn(A_x, A_wqkv, A_wo, B_x, B_w_gate, B_w_up, B_w_down)
```

```python
import jax
import jax.numpy as jnp
from jax import lax
import jax.experimental.pallas as pl
import jax.experimental.pallas.tpu as pltpu

S, D, DH, W, DIL, DF = 2048, 512, 16, 8, 2, 1376
HALO = 16
T0, LS = 512, 256
TB = 256
TL, UNROLL = 192, 4
CHUNKS = ((0, 128), (128, 256), (384, 640), (1024, 352))
GW = 384
SEC = (0, 2, 1)
LOG2E = 1.4426950408889634
F32, BF16, U32 = jnp.float32, jnp.bfloat16, jnp.uint32
NT = (((1,), (1,)), ((), ()))


def _cat(xs):
    return jnp.concatenate(xs, axis=1)


def _tree(xs, f):
    xs = list(xs)
    while len(xs) > 1:
        xs = [f(xs[i], xs[i + 1]) for i in range(0, len(xs), 2)]
    return xs[0]


def _kernel(x_hbm, wqkv_hbm, wo_hbm, wg_hbm, wu_hbm, wd_hbm, o_hbm,
            x_buf, o_buf, xn_a, xn_b, h_buf, wqkv_raw, wqkv_t, wo_raw, wo_p, st0, st1, st2, st3,
            wg_v, wu_v, wd_v, q_scr, k_scr, v_scr, sems):
    def rows(src, dst, a, n):
        return src.at[pl.ds(a, n)], dst.at[pl.ds(a, n)]

    def copies(sem, pairs):
        return [pltpu.make_async_copy(a, b, sems.at[sem]) for a, b in pairs]

    def out_copy(r, n):
        return pltpu.make_async_copy(o_buf.at[pl.ds(r, n)], o_hbm.at[pl.ds(r, n)], sems.at[7])

    def wait(group):
        for c in group:
            c.wait()

    x0_cp = copies(0, [rows(x_hbm, x_buf, 0, T0)])
    chunk_cp = [copies(1 + i, [rows(wg_hbm, wg_v, a, m), rows(wu_hbm, wu_v, a, m)])
                for i, (a, m) in enumerate(CHUNKS)]
    wqkv_cp = copies(5, [(wqkv_hbm, wqkv_raw)])
    rest_cp = copies(6, [(wo_hbm, wo_raw), (wd_hbm, wd_v), rows(x_hbm, x_buf, T0, S - T0)])
    for group in [x0_cp] + chunk_cp + [wqkv_cp, rest_cp]:
        for c in group:
            c.start()

    def layernorm(r, n, xn, l):
        x = x_buf[pl.ds(r, n), :].astype(F32)
        xc = x - jnp.sum(x, axis=-1, keepdims=True) * (1.0 / D)
        var = jnp.sum(xc * xc, axis=-1, keepdims=True) * (1.0 / D)
        xn[pl.ds(l, n), :] = (xc * lax.rsqrt(var + 1e-5)).astype(BF16)

    def geglu(xn, l, n, a, m):
        x = xn[pl.ds(l, n), :]
        for c in range(a, a + m, GW):
            mm = min(GW, a + m - c)
            g = lax.dot_general(x, wg_v[pl.ds(c, mm), :], NT, preferred_element_type=F32)
            u = lax.dot_general(x, wu_v[pl.ds(c, mm), :], NT, preferred_element_type=F32)
            inner = g * (0.7978845608028654 + (0.7978845608028654 * 0.044715) * (g * g))
            th = jnp.tanh(inner)
            hg = 0.5 * g
            h_buf[pl.ds(l, n), pl.ds(c, mm)] = ((hg + hg * th) * u).astype(BF16)

    def permute_rows(w, dst, base, stage):
        wv = pltpu.bitcast(w, U32)
        for j in range(4):
            stage[j] = wv[:, 128 * j:128 * (j + 1)]
        for e in range(8):
            a = _cat([stage[j, pl.ds(e, 16, stride=16), :] for j in range(4)])
            b = _cat([stage[j, pl.ds(8 + e, 16, stride=16), :] for j in range(4)])
            lo = (a & 0xFFFF) | (b << 16)
            hi = lax.shift_right_logical(a, U32(16)) | (b & U32(0xFFFF0000))
            dst[pl.ds(base + 64 * e, 32), :] = pltpu.bitcast(lo, BF16)
            dst[pl.ds(base + 64 * e + 32, 32), :] = pltpu.bitcast(hi, BF16)

    def qkv(xn, l, n, first=False):
        r = lax.dot_general(xn[pl.ds(l, n), :], wqkv_t[...], NT, preferred_element_type=F32)
        oq, ok, ov = (D * s for s in SEC)
        for j in range(4):
            q_scr[j, pl.ds(l, n), :] = r[:, oq + 128 * j:oq + 128 * (j + 1)] * (DH ** -0.5 * LOG2E)
            k_scr[j, pl.ds(HALO + l, n), :] = r[:, ok + 128 * j:ok + 128 * (j + 1)]
            v_scr[j, pl.ds(HALO + l, n), :] = r[:, ov + 128 * j:ov + 128 * (j + 1)]
        if first:
            for j in range(4):
                k_scr[j, 0:HALO, :] = jnp.zeros((HALO, 128), F32)
                v_scr[j, 0:HALO, :] = jnp.broadcast_to(
                    r[0:1, ov + 128 * j:ov + 128 * (j + 1)], (HALO, 128))

    def keep_halo(l):
        for j in range(4):
            k_scr[j, 0:HALO, :] = k_scr[j, pl.ds(l, HALO), :]
            v_scr[j, 0:HALO, :] = v_scr[j, pl.ds(l, HALO), :]

    def attention(l, n, first=False):
        q = [q_scr[j, pl.ds(l, n), :] for j in range(4)]
        logits = []
        for w in range(W):
            off = HALO + l - DIL * w
            s = _tree([q[j] * k_scr[j, pl.ds(off, n), :] for j in range(4)], jnp.add)
            s = s + pltpu.roll(s, 64, 1)
            s = s + pltpu.roll(s, 32, 1)
            if first and w > 0:
                pos = lax.broadcasted_iota(jnp.int32, (HALO, 128), 0)
                s = jnp.concatenate(
                    [jnp.where(pos >= DIL * w, s[0:HALO], -1e9 * LOG2E), s[HALO:]], axis=0)
            logits.append(s)
        m = _tree(logits, jnp.maximum)
        e = [jnp.exp2(s - m) for s in logits]
        inv = 1.0 / _tree(e, jnp.add)
        out = []
        for j in range(4):
            acc = e[0] * v_scr[j, pl.ds(HALO + l, n), :]
            for w in range(1, W):
                acc = acc + e[w] * v_scr[j, pl.ds(HALO + l - DIL * w, n), :]
            out.append((acc * inv).astype(BF16))
        return _cat(out)

    def finish(r, n, l, o):
        acc = x_buf[pl.ds(r, n), :].astype(F32)
        acc = acc + jnp.dot(h_buf[pl.ds(l, n), :], wd_v[...], preferred_element_type=F32)
        acc = acc + jnp.dot(o, wo_p[...], preferred_element_type=F32)
        o_buf[pl.ds(r, n), :] = acc.astype(BF16)

    wait(x0_cp)
    layernorm(0, LS, xn_a, 0)
    for i, (a, m) in enumerate(CHUNKS):
        wait(chunk_cp[i])
        if i == 0:
            layernorm(LS, T0 - LS, xn_a, LS)
            geglu(xn_a, 0, LS, a, m)
            geglu(xn_a, LS, T0 - LS, a, m)
        else:
            if i == len(CHUNKS) - 1:
                wait(wqkv_cp)
            geglu(xn_a, 0, T0, a, m)
    for s, stage in enumerate((st0, st1, st2)):
        permute_rows(wqkv_raw[:, pl.ds(D * s, D)].T, wqkv_t, D * SEC[s], stage)
    qkv(xn_a, 0, TB, first=True)
    wait(rest_cp)
    permute_rows(wo_raw[...], wo_p, 0, st3)
    for l in range(TB, T0, TB):
        qkv(xn_a, l, TB)
    outs = [attention(l, TB, first=(l == 0)) for l in range(0, T0, TB)]
    keep_halo(T0)
    layernorm(T0, TL, xn_a, 0)
    for l, o in zip(range(0, T0, TB), outs):
        finish(l, TB, l, o)
    out_copy(0, T0).start()

    def body(i, carry):
        r0 = pl.multiple_of(T0 + i * (TL * UNROLL), 64)
        for t in range(UNROLL):
            xn, xn_next = (xn_a, xn_b) if t % 2 == 0 else (xn_b, xn_a)
            r = pl.multiple_of(r0 + t * TL, 16)
            qkv(xn, 0, TL)
            o = attention(0, TL)
            geglu(xn, 0, TL, 0, DF)
            layernorm(pl.multiple_of(jnp.minimum(r0 + (t + 1) * TL, S - TL), 16), TL, xn_next, 0)
            keep_halo(TL)
            finish(r, TL, 0, o)
            out_copy(r, TL).start()
        return carry

    n_tiles = (S - T0) // TL
    lax.fori_loop(0, n_tiles // UNROLL, body, 0)
    out_copy(0, T0).wait()
    for t in range(n_tiles):
        out_copy(T0 + t * TL, TL).wait()


@jax.jit
def pallas_parallel_sum__sliding_local_dilated__glu_gated_geglu__prompt_kernel(
    A_x: jax.Array,
    A_wqkv: jax.Array,
    A_wo: jax.Array,
    B_x: jax.Array,
    B_w_gate: jax.Array,
    B_w_up: jax.Array,
    B_w_down: jax.Array,
):
    del B_x
    hbm = pl.BlockSpec(memory_space=pltpu.HBM)
    out = pl.pallas_call(
        _kernel,
        in_specs=[hbm] * 6,
        out_specs=hbm,
        out_shape=jax.ShapeDtypeStruct((S, D), A_x.dtype),
        scratch_shapes=[
            pltpu.VMEM((S, D), BF16), pltpu.VMEM((S, D), BF16),
            pltpu.VMEM((T0, D), BF16), pltpu.VMEM((T0, D), BF16),
            pltpu.VMEM((T0, DF), BF16),
            pltpu.VMEM((D, 3 * D), BF16), pltpu.VMEM((3 * D, D), BF16),
            pltpu.VMEM((D, D), BF16), pltpu.VMEM((D, D), BF16),
            *([pltpu.VMEM((4, D // 2, 128), U32)] * 4),
            *([pltpu.VMEM((DF, D), BF16)] * 3),
            pltpu.VMEM((4, T0, 128), F32),
            pltpu.VMEM((4, HALO + T0, 128), F32),
            pltpu.VMEM((4, HALO + T0, 128), F32),
            pltpu.SemaphoreType.DMA((8,)),
        ],
        compiler_params=pltpu.CompilerParams(
            vmem_limit_bytes=100 * 1024 * 1024,
            flags={"XLA_TPU_EVENLY_DISTRIBUTE_CRITICAL_NODES": True},
        ),
    )(A_x.reshape(S, D), A_wqkv, A_wo, B_w_gate.T, B_w_up.T, B_w_down)
    return out.reshape(1, S, D)
```
